```python
import jax
import jax.numpy as jnp

def _softmax(x, axis=-1):
    return jax.nn.softmax(x, axis=axis)
def _gelu(x):
    return jax.nn.gelu(x, approximate=True)
def _silu(x):
    return jax.nn.silu(x)
def _sigmoid(x):
    return jax.nn.sigmoid(x)
def _layernorm(x, axis=-1, eps=1e-5):
    m = jnp.mean(x, axis=axis, keepdims=True)
    v = jnp.var(x, axis=axis, keepdims=True)
    return (x - m) / jnp.sqrt(v + eps)
def _scatter_add(tgt, idx, src, axis=0):
    return tgt.at[idx].add(src)
def _segment_sum(src, seg, n):
    return jax.ops.segment_sum(src, seg, n)
class _Rng:
    def __init__(self, key):
        self._k = key
    def _next(self):
        self._k, sub = jax.random.split(self._k)
        return sub
    def normal(self, shape):
        return jax.random.normal(self._next(), shape, dtype=jnp.bfloat16)
    def randint(self, lo, hi, shape):
        return jax.random.randint(self._next(), shape, lo, hi, dtype=jnp.int32)
    def uniform(self, shape, lo=0.0, hi=1.0):
        return jax.random.uniform(self._next(), shape, jnp.bfloat16, lo, hi)
    def permutation(self, n):
        return jax.random.permutation(self._next(), n)


kernel_name = 'sequential_preLN__compressed_kv_cla__moe_arch_mod__decode'

def setup_inputs():
    _rng = _Rng(jax.random.key(int.from_bytes(__import__("os").urandom(4), "little")))
    _w = (lambda a: (lambda t: t.astype(jnp.bfloat16) if jnp.issubdtype(t.dtype, jnp.floating) else t)(jnp.asarray(a)))
    def _A_setup():
        B, H, Sq, Sk, D, M = 1, 32, 1, 8192, 128, 512
        Dc = 4 * D
        return {
            "x": _w((lambda *s: _rng.normal(s) * 0.05)(B, Sq, M)),
            "c_kv": _w((lambda *s: _rng.normal(s) * 0.05)(B, Sk, Dc)),
            "w_q": _w((lambda *s: _rng.normal(s) * 0.05)(M, H, D) * (M ** -0.5)),
            "w_uk": _w((lambda *s: _rng.normal(s) * 0.05)(Dc, H, D) * (Dc ** -0.5)),
            "w_uv": _w((lambda *s: _rng.normal(s) * 0.05)(Dc, H, D) * (Dc ** -0.5)),
            "w_o": _w((lambda *s: _rng.normal(s) * 0.05)(H, D, M) * ((H * D) ** -0.5)),
        }
    _A_in = _A_setup()

    def _B_setup():
        B, S, D, F, C = 1, 1, 512, 1376, 1
        return {
            "x": _w((lambda *s: _rng.normal(s) * 0.05)(B, S, D)),
            "w_r": _w((lambda *s: _rng.normal(s) * 0.05)(D)),
            "w_gate": _w((lambda *s: _rng.normal(s) * 0.05)(D, F)),
            "w_up": _w((lambda *s: _rng.normal(s) * 0.05)(D, F)),
            "w_down": _w((lambda *s: _rng.normal(s) * 0.05)(F, D)),
        }
    _B_in = _B_setup()

    return {
        "A_x": _A_in["x"],
        "A_c_kv": _A_in["c_kv"],
        "A_w_q": _A_in["w_q"],
        "A_w_uk": _A_in["w_uk"],
        "A_w_uv": _A_in["w_uv"],
        "A_w_o": _A_in["w_o"],
        "B_x": _B_in["x"],
        "B_w_r": _B_in["w_r"],
        "B_w_gate": _B_in["w_gate"],
        "B_w_up": _B_in["w_up"],
        "B_w_down": _B_in["w_down"],
    }

def reference(A_x, A_c_kv, A_w_q, A_w_uk, A_w_uv, A_w_o, B_x, B_w_r, B_w_gate, B_w_up, B_w_down):
    def _A_ref(x, c_kv, w_q, w_uk, w_uv, w_o):
        B, Sq, M = x.shape[0], x.shape[1], x.shape[2]
        Sk = c_kv.shape[1]
        H, D = w_q.shape[1], w_q.shape[2]
        q = jnp.einsum("bqm,mhd->bhqd", x, w_q)
        k = jnp.einsum("bkc,chd->bhkd", c_kv, w_uk)
        v = jnp.einsum("bkc,chd->bhkd", c_kv, w_uv)
        scores = jnp.einsum("bhqd,bhkd->bhqk", q, k) * (D ** -0.5)
        off = Sk - Sq
        qi = jnp.arange(Sq)[:, None]
        kj = jnp.arange(Sk)[None, :]
        cmask = kj <= (qi + off)
        scores = jnp.where(cmask[None, None], scores, -1e9)
        p = _softmax(scores, axis=-1)
        ctx = jnp.einsum("bhqk,bhkd->bhqd", p, v)
        return jnp.einsum("bhqd,hdm->bqm", ctx, w_o)

    def _B_ref(x, w_r, w_gate, w_up, w_down):
        B, S, D = x.shape
        C = 1
        r = x @ w_r
        idx = jnp.argsort(-r, axis=-1)[:, :C]
        idx_e = jnp.repeat(idx.reshape(B, C, 1), D, axis=2)
        x_sel = jnp.take_along_axis(x, idx_e, axis=1)
        g = _silu(x_sel @ w_gate)
        u = x_sel @ w_up
        y = (g * u) @ w_down
        r_sel = _sigmoid(jnp.take_along_axis(r, idx, axis=1))
        y = y * r_sel.reshape(B, C, 1)
        b_off = (jnp.arange(B) * S).reshape(B, 1)
        flat_idx = (idx + b_off).reshape(B * C)
        zero = (x * 0.0).reshape(B * S, D)
        upd = _scatter_add(zero, flat_idx, y.reshape(B * C, D), axis=0)
        return x + upd.reshape(B, S, D)

    x = A_x
    h = x + _A_ref(_layernorm(x, axis=-1), A_c_kv, A_w_q, A_w_uk, A_w_uv, A_w_o)
    h2 = h + _B_ref(_layernorm(h, axis=-1), B_w_r, B_w_gate, B_w_up, B_w_down)
    return h2
```

```python
import jax
import jax.numpy as jnp
from jax import lax
import jax.experimental.pallas as pl
import jax.experimental.pallas.tpu as pltpu

_EPS = 1e-5
_LANES = 128
_NT = (((1,), (1,)), ((), ()))

_KV_BLOCK = 512
_HEAD_UNROLL = 8
_FFN_UNROLL = 4
_DOWN_TAIL = (384, 128)
_N_SEM = 3


def _down_pieces(F):
    whole = F // _LANES * _LANES
    return (whole - sum(_DOWN_TAIL), *_DOWN_TAIL, F - whole)


def _layernorm(v):
    mean = jnp.mean(v, axis=-1, keepdims=True)
    cen = v - mean
    var = jnp.mean(cen * cen, axis=-1, keepdims=True)
    return cen / jnp.sqrt(var + _EPS)


def _sigmoid(v):
    return 1.0 / (1.0 + jnp.exp(-v))


def _kernel(x_hbm, ckv_hbm, wq_hbm, wuk_hbm, wuv_hbm, wo_hbm, wr_hbm, wg_hbm, wu_hbm, wd_hbm,
            out_hbm,
            x_v, ckv_v, wq_v, wuk_v, wuv_v, wo_v, wr_v, wg_v, wu_v, wd_v, out_v,
            xb_v, tr_v, s_v, ctx_v, g_v, act_v, y_v, sems):
    f32, bf16 = jnp.float32, jnp.bfloat16
    M, H, D = wq_v.shape
    Sk, Dc = ckv_v.shape
    F = wd_v.shape[0]

    stream = [[(wq_hbm, wq_v), (x_hbm, x_v)], [(wuk_hbm, wuk_v)], [(ckv_hbm, ckv_v)],
              [(wuv_hbm, wuv_v)], [(wo_hbm, wo_v)], [(wg_hbm, wg_v), (wr_hbm, wr_v)],
              [(wu_hbm, wu_v)]]
    down_pieces, start = _down_pieces(F), 0
    for rows in down_pieces:
        stream.append([(wd_hbm.at[pl.ds(start, rows)], wd_v.at[pl.ds(start, rows)])])
        start += rows
    stream = [[pltpu.make_async_copy(src, dst, sems.at[i % _N_SEM]) for src, dst in entry]
              for i, entry in enumerate(stream)]
    for entry in stream[:_N_SEM]:
        for cp in entry:
            cp.start()
    arrived = 0

    def wait_next():
        nonlocal arrived
        with jax.named_scope(f"w{arrived}"):
            for cp in stream[arrived]:
                cp.wait()
            if arrived + _N_SEM < len(stream):
                for cp in stream[arrived + _N_SEM]:
                    cp.start()
        arrived += 1

    wait_next()
    with jax.named_scope("q"):
        x = x_v[0].astype(f32)
        xn = _layernorm(x)
        for j in range(M // _LANES):
            blk = jnp.broadcast_to(xn[:, j * _LANES:(j + 1) * _LANES], (_LANES, _LANES))
            xb_v[j * _LANES:(j + 1) * _LANES, :] = blk.T

        def q_step(m, acc):
            return acc + wq_v[m].astype(f32) * xb_v[pl.ds(m, 1), :]

        q = lax.fori_loop(0, M, q_step, jnp.zeros((H, D), f32), unroll=8)
        q = q * (D ** -0.5)

    n_grp = Dc // _LANES
    own_head = (lax.broadcasted_iota(jnp.int32, (H, _LANES), 0)
                == lax.broadcasted_iota(jnp.int32, (H, _LANES), 1) % H)

    def head_tile(w_ref, t):
        return jnp.concatenate([w_ref[t + j * _LANES] for j in range(n_grp)], axis=0)

    wait_next()
    with jax.named_scope("qa"):
        qb = q.astype(bf16)

        def qa_step(t, carry):
            prod = lax.dot_general(qb, head_tile(wuk_v, t), _NT, preferred_element_type=f32)
            tr_v[pl.ds(t, 1), :] = jnp.sum(jnp.where(own_head, prod, 0.0), axis=0, keepdims=True)
            return carry

        lax.fori_loop(0, _LANES, qa_step, 0, unroll=_HEAD_UNROLL)
        qa_t = tr_v[...].T
        qa = jnp.concatenate([qa_t[j * H:(j + 1) * H] for j in range(n_grp)], axis=-1).astype(bf16)

    wait_next()
    n_kv = Sk // _KV_BLOCK
    with jax.named_scope("scores"):
        def score_step(b, mx):
            rows = pl.ds(pl.multiple_of(b * _KV_BLOCK, _KV_BLOCK), _KV_BLOCK)
            s = lax.dot_general(qa, ckv_v[rows, :], _NT, preferred_element_type=f32)
            s_v[b] = s
            for j in range(_KV_BLOCK // _LANES):
                mx = jnp.maximum(mx, s[:, j * _LANES:(j + 1) * _LANES])
            return mx

        mx = lax.fori_loop(0, n_kv, score_step, jnp.full((H, _LANES), -jnp.inf, f32))
        mx = jnp.max(mx, axis=-1, keepdims=True)

    with jax.named_scope("pv"):
        def pv_step(b, carry):
            den, acc = carry
            rows = pl.ds(pl.multiple_of(b * _KV_BLOCK, _KV_BLOCK), _KV_BLOCK)
            p = jnp.exp(s_v[b] - mx)
            for j in range(_KV_BLOCK // _LANES):
                den = den + p[:, j * _LANES:(j + 1) * _LANES]
            acc = acc + jnp.dot(p.astype(bf16), ckv_v[rows, :], preferred_element_type=f32)
            return den, acc

        den, acc = lax.fori_loop(0, n_kv, pv_step,
                                 (jnp.zeros((H, _LANES), f32), jnp.zeros((H, Dc), f32)))
        cc = acc / jnp.sum(den, axis=-1, keepdims=True)
        cc_t = jnp.concatenate([cc[:, j * _LANES:(j + 1) * _LANES] for j in range(n_grp)], axis=0)
        tr_v[...] = cc_t.T

    wait_next()
    with jax.named_scope("ctx"):
        def ctx_step(t, acc):
            coef = jnp.where(own_head, tr_v[pl.ds(t, 1), :], 0.0).astype(bf16)
            return acc + jnp.dot(coef, head_tile(wuv_v, t), preferred_element_type=f32)

        ctx_v[...] = lax.fori_loop(0, _LANES, ctx_step, jnp.zeros((H, D), f32), unroll=_HEAD_UNROLL)

    wait_next()
    with jax.named_scope("o"):
        def o_step(h, acc):
            row = jnp.broadcast_to(ctx_v[pl.ds(h, 1), :], (8, D)).astype(bf16)
            return acc + jnp.dot(row, wo_v[h], preferred_element_type=f32)

        attn = lax.fori_loop(0, H, o_step, jnp.zeros((8, M), f32), unroll=4)
        h1 = x + attn[0:1]
        hn = _layernorm(h1)
        hb = jnp.broadcast_to(hn, (8, M)).astype(bf16)

    n_full = F // _LANES
    rem = F - n_full * _LANES
    def project(w_ref, dst_ref):
        def step(j, carry):
            start = pl.multiple_of(jnp.minimum(j * _LANES, F - _LANES), 16)
            dst_ref[j] = lax.dot_general(hb, w_ref[pl.ds(start, _LANES), :], _NT,
                                         preferred_element_type=f32)
            return carry

        lax.fori_loop(0, dst_ref.shape[0], step, 0, unroll=_FFN_UNROLL)

    wait_next()
    with jax.named_scope("g"):
        project(wg_v, g_v)
    wait_next()
    with jax.named_scope("u"):
        project(wu_v, act_v)
    with jax.named_scope("act"):
        wr = wr_v[...].astype(f32)
        r = jnp.zeros((1, _LANES), f32)
        for j in range(M // _LANES):
            r = r + hn[:, j * _LANES:(j + 1) * _LANES] * wr[j:j + 1]
        route = _sigmoid(jnp.sum(r, axis=-1, keepdims=True))
        g = g_v[...]
        act = g * _sigmoid(g) * act_v[...] * route
        act_v[...] = act
        act_col = jnp.broadcast_to(act[n_full, 0:1], (_LANES, _LANES)).T[_LANES - rem:]
        y_v[...] = jnp.broadcast_to(h1 + (hn + hn * 0.0), (8, M))

    start = 0
    for rows in down_pieces[:-1]:
        wait_next()
        with jax.named_scope("d"):
            groups = range(start // _LANES, (start + rows) // _LANES)
            lhs = jnp.concatenate([act_v[j] for j in groups], axis=-1).astype(bf16)
            y_v[...] += jnp.dot(lhs, wd_v[start:start + rows, :], preferred_element_type=f32)
        start += rows

    first_row = lax.broadcasted_iota(jnp.int32, (8, M), 0) == 0
    y = jnp.where(first_row, y_v[...], 0.0)
    wait_next()
    with jax.named_scope("out"):
        w_tail = wd_v[start:, :].astype(f32)
        parts = []
        for j in range(M // _LANES):
            prod = w_tail[:, j * _LANES:(j + 1) * _LANES] * act_col
            parts.append(jnp.sum(prod.reshape(rem // 8, 8, _LANES), axis=0))
        y = y + jnp.concatenate(parts, axis=-1)
        out_v[0] = jnp.sum(y, axis=0, keepdims=True).astype(out_v.dtype)
        cp_out = pltpu.make_async_copy(out_v, out_hbm, sems.at[arrived % _N_SEM])
        cp_out.start()
        cp_out.wait()


@jax.jit
def pallas_sequential_preLN__compressed_kv_cla__moe_arch_mod__decode_kernel(
    A_x: jax.Array,
    A_c_kv: jax.Array,
    A_w_q: jax.Array,
    A_w_uk: jax.Array,
    A_w_uv: jax.Array,
    A_w_o: jax.Array,
    B_x: jax.Array,
    B_w_r: jax.Array,
    B_w_gate: jax.Array,
    B_w_up: jax.Array,
    B_w_down: jax.Array,
):
    del B_x
    B, Sq, M = A_x.shape
    _, Sk, Dc = A_c_kv.shape
    _, H, D = A_w_q.shape
    F = B_w_down.shape[0]
    assert B == 1 and Sq == 1 and D == _LANES
    assert F % _LANES and F % 16 == 0

    operands = (A_x, A_c_kv.reshape(Sk, Dc), A_w_q, A_w_uk, A_w_uv, A_w_o,
                B_w_r.reshape(M // _LANES, _LANES), B_w_gate.T, B_w_up.T, B_w_down)
    f32 = jnp.float32
    n_grp = pl.cdiv(pl.cdiv(F, _LANES), _FFN_UNROLL) * _FFN_UNROLL
    scratch = [pltpu.VMEM(a.shape, a.dtype) for a in operands] + [
        pltpu.VMEM(A_x.shape, A_x.dtype),
        pltpu.VMEM((M, _LANES), f32),
        pltpu.VMEM((_LANES, _LANES), f32),
        pltpu.VMEM((Sk // _KV_BLOCK, H, _KV_BLOCK), f32),
        pltpu.VMEM((H, D), f32),
        pltpu.VMEM((n_grp, 8, _LANES), f32),
        pltpu.VMEM((n_grp, 8, _LANES), f32),
        pltpu.VMEM((8, M), f32),
        pltpu.SemaphoreType.DMA((_N_SEM,)),
    ]
    return pl.pallas_call(
        _kernel,
        out_shape=jax.ShapeDtypeStruct(A_x.shape, A_x.dtype),
        in_specs=[pl.BlockSpec(memory_space=pltpu.HBM)] * len(operands),
        out_specs=pl.BlockSpec(memory_space=pltpu.HBM),
        scratch_shapes=scratch,
        compiler_params=pltpu.CompilerParams(vmem_limit_bytes=64 * 1024 * 1024),
    )(*operands)
```

```python
import functools

import jax
import jax.numpy as jnp
from jax import lax
import jax.experimental.pallas as pl
import jax.experimental.pallas.tpu as pltpu

_EPS = 1e-5
_LANES = 128
_NT = (((1,), (1,)), ((), ()))

_KV_BLOCK = 1024
_HEAD_UNROLL = 8
_FFN_UNROLL = 4
_DOWN_MXU = (256, 128)


def _layernorm(v):
    mean = jnp.mean(v, axis=-1, keepdims=True)
    cen = v - mean
    var = jnp.mean(cen * cen, axis=-1, keepdims=True)
    return cen / jnp.sqrt(var + _EPS)


def _sigmoid(v):
    return 1.0 / (1.0 + jnp.exp(-v))


def _lane_groups(v):
    return [v[:, j:j + _LANES] for j in range(0, v.shape[-1], _LANES)]


def _down_pieces(F):
    whole = F // _LANES * _LANES
    return (whole - sum(_DOWN_MXU), *_DOWN_MXU, F - whole)


def _block(x_hbm, ckv_hbm, wq_hbm, wuk_hbm, wuv_hbm, wo_hbm, wr_hbm, wg_hbm, wu_hbm, wd_hbm,
           x_v, ckv_v, wq_v, wuk_v, wuv_v, wo_v, wr_v, wg_v, wu_v, wd_v,
           xb_v, tr_v, s_v, ctx_v, g_v, act_v, y_v, out_v, sems):
    f32, bf16 = jnp.float32, jnp.bfloat16
    M, H, D = wq_v.shape
    Sk, Dc = ckv_v.shape
    F = wd_v.shape[0]

    pairs = [(x_hbm, x_v), (wq_hbm, wq_v), (wuk_hbm, wuk_v), (ckv_hbm, ckv_v), (wuv_hbm, wuv_v),
             (wo_hbm, wo_v), (wr_hbm, wr_v), (wg_hbm, wg_v), (wu_hbm, wu_v)]
    down_pieces, start = _down_pieces(F), 0
    for rows in down_pieces:
        pairs.append((wd_hbm.at[pl.ds(start, rows)], wd_v.at[pl.ds(start, rows)]))
        start += rows
    copies = [pltpu.make_async_copy(src, dst, sems.at[i]) for i, (src, dst) in enumerate(pairs)]
    for cp in copies:
        cp.start()
    cp_x, cp_wq, cp_wuk, cp_ckv, cp_wuv, cp_wo, cp_wr, cp_wg, cp_wu, *cp_wd = copies

    cp_x.wait()
    x = x_v[0].astype(f32)
    for j, part in enumerate(_lane_groups(_layernorm(x))):
        xb_v[j * _LANES:(j + 1) * _LANES, :] = jnp.broadcast_to(part, (_LANES, _LANES)).T

    def q_step(m, acc):
        return acc + wq_v[m].astype(f32) * xb_v[pl.ds(m, 1), :]

    cp_wq.wait()
    q = lax.fori_loop(0, M, q_step, jnp.zeros((H, D), f32), unroll=8)
    q = (q * D ** -0.5).astype(bf16)

    own_head = (lax.broadcasted_iota(jnp.int32, (H, _LANES), 0)
                == lax.broadcasted_iota(jnp.int32, (H, _LANES), 1) % H)

    def head_tile(w_ref, t):
        return jnp.concatenate([w_ref[t + j] for j in range(0, Dc, _LANES)], axis=0)

    def qa_step(t, carry):
        prod = lax.dot_general(q, head_tile(wuk_v, t), _NT, preferred_element_type=f32)
        tr_v[pl.ds(t, 1), :] = jnp.sum(jnp.where(own_head, prod, 0.0), axis=0, keepdims=True)
        return carry

    cp_wuk.wait()
    lax.fori_loop(0, _LANES, qa_step, 0, unroll=_HEAD_UNROLL)
    qa_t = tr_v[...].T
    qa = jnp.concatenate([qa_t[j:j + H] for j in range(0, _LANES, H)], axis=-1).astype(bf16)

    def kv_rows(b):
        return pl.ds(pl.multiple_of(b * _KV_BLOCK, _KV_BLOCK), _KV_BLOCK)

    def score_step(b, top):
        s = lax.dot_general(qa, ckv_v[kv_rows(b), :], _NT, preferred_element_type=f32)
        s_v[b] = s
        return functools.reduce(jnp.maximum, _lane_groups(s), top)

    cp_ckv.wait()
    top = lax.fori_loop(0, Sk // _KV_BLOCK, score_step, jnp.full((H, _LANES), -jnp.inf, f32))
    top = jnp.max(top, axis=-1, keepdims=True)

    def pv_step(b, carry):
        den, acc = carry
        p = jnp.exp(s_v[b] - top)
        den = functools.reduce(jnp.add, _lane_groups(p), den)
        return den, acc + jnp.dot(p.astype(bf16), ckv_v[kv_rows(b), :], preferred_element_type=f32)

    den, acc = lax.fori_loop(0, Sk // _KV_BLOCK, pv_step,
                             (jnp.zeros((H, _LANES), f32), jnp.zeros((H, Dc), f32)))
    cc = acc / jnp.sum(den, axis=-1, keepdims=True)
    tr_v[...] = jnp.concatenate(_lane_groups(cc), axis=0).T

    def ctx_step(t, acc):
        coef = jnp.where(own_head, tr_v[pl.ds(t, 1), :], 0.0).astype(bf16)
        return acc + jnp.dot(coef, head_tile(wuv_v, t), preferred_element_type=f32)

    cp_wuv.wait()
    ctx_v[...] = lax.fori_loop(0, _LANES, ctx_step, jnp.zeros((H, D), f32), unroll=_HEAD_UNROLL)

    def out_step(h, acc):
        row = jnp.broadcast_to(ctx_v[pl.ds(h, 1), :], (8, D)).astype(bf16)
        return acc + jnp.dot(row, wo_v[h], preferred_element_type=f32)

    cp_wo.wait()
    attn = lax.fori_loop(0, H, out_step, jnp.zeros((8, M), f32), unroll=4)
    h1 = x + attn[0:1]
    hn = _layernorm(h1)
    hb = jnp.broadcast_to(hn, (8, M)).astype(bf16)

    cp_wr.wait()
    wr = wr_v[...].astype(f32)
    score = sum(part * wr[j:j + 1] for j, part in enumerate(_lane_groups(hn)))
    route = _sigmoid(jnp.sum(score, axis=-1, keepdims=True))

    def project(w_ref, dst_ref):
        def step(j, carry):
            first = pl.multiple_of(jnp.minimum(j * _LANES, F - _LANES), 16)
            dst_ref[j] = lax.dot_general(hb, w_ref[pl.ds(first, _LANES), :], _NT,
                                         preferred_element_type=f32)
            return carry

        lax.fori_loop(0, dst_ref.shape[0], step, 0, unroll=_FFN_UNROLL)

    cp_wg.wait()
    project(wg_v, g_v)
    cp_wu.wait()
    project(wu_v, act_v)
    g = g_v[...]
    act = g * _sigmoid(g) * act_v[...] * route
    act_v[...] = act
    tail = down_pieces[-1]
    act_col = jnp.broadcast_to(act[F // _LANES, 0:1], (_LANES, _LANES)).T[_LANES - tail:]
    y_v[...] = jnp.broadcast_to(h1 + (hn + hn * 0.0), (8, M))

    start = 0
    for cp, rows in zip(cp_wd, down_pieces[:-1]):
        cp.wait()
        groups = range(start // _LANES, (start + rows) // _LANES)
        lhs = jnp.concatenate([act_v[j] for j in groups], axis=-1).astype(bf16)
        y_v[...] += jnp.dot(lhs, wd_v[start:start + rows, :], preferred_element_type=f32)
        start += rows

    y = jnp.where(lax.broadcasted_iota(jnp.int32, (8, M), 0) == 0, y_v[...], 0.0)
    cp_wd[-1].wait()
    parts = [jnp.sum((w * act_col).reshape(tail // 8, 8, _LANES), axis=0)
             for w in _lane_groups(wd_v[start:, :].astype(f32))]
    y = y + jnp.concatenate(parts, axis=-1)
    out_v[0] = jnp.sum(y, axis=0, keepdims=True).astype(out_v.dtype)


def _kernel(*refs, n_in, n_copies):
    out_hbm, out_v = refs[n_in], refs[-1]

    def run(out_sem):
        pl.run_scoped(functools.partial(_block, *refs[:n_in], *refs[n_in + 1:]),
                      pltpu.SemaphoreType.DMA((n_copies,)))
        cp_out = pltpu.make_async_copy(out_v, out_hbm, out_sem)
        cp_out.start()
        cp_out.wait()

    pl.run_scoped(run, pltpu.SemaphoreType.DMA(()))


@jax.jit
def pallas_sequential_preLN__compressed_kv_cla__moe_arch_mod__decode_kernel(
    A_x: jax.Array,
    A_c_kv: jax.Array,
    A_w_q: jax.Array,
    A_w_uk: jax.Array,
    A_w_uv: jax.Array,
    A_w_o: jax.Array,
    B_x: jax.Array,
    B_w_r: jax.Array,
    B_w_gate: jax.Array,
    B_w_up: jax.Array,
    B_w_down: jax.Array,
):
    del B_x
    B, Sq, M = A_x.shape
    _, Sk, Dc = A_c_kv.shape
    _, H, D = A_w_q.shape
    F = B_w_down.shape[0]
    assert B == 1 and Sq == 1 and D == _LANES and H * (Dc // _LANES) == _LANES
    assert Sk % _KV_BLOCK == 0 and M % _LANES == 0 and F % _LANES and F % 16 == 0

    operands = (A_x, A_c_kv.reshape(Sk, Dc), A_w_q, A_w_uk, A_w_uv, A_w_o,
                B_w_r.reshape(M // _LANES, _LANES), B_w_gate.T, B_w_up.T, B_w_down)
    f32 = jnp.float32
    groups = pl.cdiv(pl.cdiv(F, _LANES), _FFN_UNROLL) * _FFN_UNROLL
    scratch = [pltpu.VMEM(a.shape, a.dtype) for a in operands] + [
        pltpu.VMEM((M, _LANES), f32),
        pltpu.VMEM((_LANES, _LANES), f32),
        pltpu.VMEM((Sk // _KV_BLOCK, H, _KV_BLOCK), f32),
        pltpu.VMEM((H, D), f32),
        pltpu.VMEM((groups, 8, _LANES), f32),
        pltpu.VMEM((groups, 8, _LANES), f32),
        pltpu.VMEM((8, M), f32),
        pltpu.VMEM(A_x.shape, A_x.dtype),
    ]
    n_copies = len(operands) - 1 + len(_down_pieces(F))
    return pl.pallas_call(
        functools.partial(_kernel, n_in=len(operands), n_copies=n_copies),
        out_shape=jax.ShapeDtypeStruct(A_x.shape, A_x.dtype),
        in_specs=[pl.BlockSpec(memory_space=pltpu.HBM)] * len(operands),
        out_specs=pl.BlockSpec(memory_space=pltpu.HBM),
        scratch_shapes=scratch,
        compiler_params=pltpu.CompilerParams(vmem_limit_bytes=64 * 1024 * 1024),
    )(*operands)
```
